```python
import os as _os
_os.environ.setdefault("JAX_PLATFORMS", "cpu")
import jax
import jax.numpy as jnp

def _softmax(x, axis=-1):
    return jax.nn.softmax(x, axis=axis)
def _gelu(x):
    return jax.nn.gelu(x, approximate=True)
def _silu(x):
    return jax.nn.silu(x)
def _sigmoid(x):
    return jax.nn.sigmoid(x)
def _layernorm(x, axis=-1, eps=1e-5):
    m = jnp.mean(x, axis=axis, keepdims=True)
    v = jnp.var(x, axis=axis, keepdims=True)
    return (x - m) / jnp.sqrt(v + eps)
def _scatter_add(tgt, idx, src, axis=0):
    return tgt.at[idx].add(src)
def _segment_sum(src, seg, n):
    return jax.ops.segment_sum(src, seg, n)
class _Rng:
    def __init__(self, key):
        self._k = key
    def _next(self):
        self._k, sub = jax.random.split(self._k)
        return sub
    def normal(self, shape):
        return jax.random.normal(self._next(), shape, dtype=jnp.bfloat16)
    def randint(self, lo, hi, shape):
        return jax.random.randint(self._next(), shape, lo, hi, dtype=jnp.int32)
    def uniform(self, shape, lo=0.0, hi=1.0):
        return jax.random.uniform(self._next(), shape, jnp.bfloat16, lo, hi)
    def permutation(self, n):
        return jax.random.permutation(self._next(), n)


kernel_name = 'concat_heads__mha_block_cached__mha_block_cached__near_ridge'

def setup_inputs():
    _rng = _Rng(jax.random.key(int.from_bytes(__import__("os").urandom(4), "little")))
    _w = (lambda a: (lambda t: t.astype(jnp.bfloat16) if jnp.issubdtype(t.dtype, jnp.floating) else t)(jnp.asarray(a)))
    def _A_setup():
        B, Sq, D = 16, 192, 512
        H, Sk, Dh = 32, 512, 128
        return {
            "x": _w((lambda *s: _rng.normal(s) * 0.8)(B, Sq, D)),
            "k_cache": _w((lambda *s: _rng.normal(s) * 0.8)(B, H, Sk, Dh)),
            "v_cache": _w((lambda *s: _rng.normal(s) * 0.05)(B, H, Sk, Dh)),
            "wq": _w((lambda *s: _rng.normal(s) * 0.8)(D, H * Dh) * (D ** -0.5)),
            "wo": _w((lambda *s: _rng.normal(s) * 0.05)(H * Dh, D) * ((H * Dh) ** -0.5)),
        }
    _A_in = _A_setup()

    def _B_setup():
        B, Sq, D = 16, 192, 512
        H, Sk, Dh = 32, 512, 128
        return {
            "x": _w((lambda *s: _rng.normal(s) * 0.8)(B, Sq, D)),
            "k_cache": _w((lambda *s: _rng.normal(s) * 0.8)(B, H, Sk, Dh)),
            "v_cache": _w((lambda *s: _rng.normal(s) * 0.05)(B, H, Sk, Dh)),
            "wq": _w((lambda *s: _rng.normal(s) * 0.8)(D, H * Dh) * (D ** -0.5)),
            "wo": _w((lambda *s: _rng.normal(s) * 0.05)(H * Dh, D) * ((H * Dh) ** -0.5)),
        }
    _B_in = _B_setup()

    return {
        "A_x": _A_in["x"],
        "A_k_cache": _A_in["k_cache"],
        "A_v_cache": _A_in["v_cache"],
        "A_wq": _A_in["wq"],
        "A_wo": _A_in["wo"],
        "B_x": _B_in["x"],
        "B_k_cache": _B_in["k_cache"],
        "B_v_cache": _B_in["v_cache"],
        "B_wq": _B_in["wq"],
        "B_wo": _B_in["wo"],
    }

def reference(A_x, A_k_cache, A_v_cache, A_wq, A_wo, B_x, B_k_cache, B_v_cache, B_wq, B_wo):
    def _A_ref(x, k_cache, v_cache, wq, wo):
        B, Sq, D = x.shape
        H, Dh = 32, 128
        q = (lambda x, *d: x.transpose(*d))((x @ wq).reshape(B, Sq, H, Dh), 0, 2, 1, 3)
        scores = jnp.einsum("bhqd,bhkd->bhqk", q, k_cache) * (Dh ** -0.5)
        p = _softmax(scores, axis=-1)
        o = jnp.einsum("bhqk,bhkd->bhqd", p, v_cache)
        return (lambda x, *d: x.transpose(*d))(o, 0, 2, 1, 3).reshape(B, Sq, H * Dh) @ wo

    def _B_ref(x, k_cache, v_cache, wq, wo):
        B, Sq, D = x.shape
        H, Dh = 32, 128
        q = (lambda x, *d: x.transpose(*d))((x @ wq).reshape(B, Sq, H, Dh), 0, 2, 1, 3)
        scores = jnp.einsum("bhqd,bhkd->bhqk", q, k_cache) * (Dh ** -0.5)
        p = _softmax(scores, axis=-1)
        o = jnp.einsum("bhqk,bhkd->bhqd", p, v_cache)
        return (lambda x, *d: x.transpose(*d))(o, 0, 2, 1, 3).reshape(B, Sq, H * Dh) @ wo

    a = _A_ref(A_x, A_k_cache, A_v_cache, A_wq, A_wo)
    b = _B_ref(B_x, B_k_cache, B_v_cache, B_wq, B_wo)
    return jnp.concatenate([a, b], axis=-1)
```

```python
import functools
import jax
import jax.numpy as jnp
from jax import lax
import jax.experimental.pallas as pl
import jax.experimental.pallas.tpu as pltpu

LOG2E = 1.4426950408889634
bf16 = jnp.bfloat16
f32 = jnp.float32

def make(SP=3, qlead=0, rcp="div", prenorm=False, nobounds=True, C=4, NB=8, SM=2, dims=None, interpret=False):
    B, SQ, D, H, SK, DH = dims or (16, 192, 512, 32, 512, 128)
    NG = H // C
    NH = B // NB
    assert NH == 2 and SP in (2, 3)
    NS = NG * NH
    CW = C * DH
    HB = NB // SM
    SPB = 2 * HB
    NSM = SP * SPB
    c = (DH ** -0.5) * LOG2E

    def kernel(ax, ak, av, awq, awo, bx, bk, bv, bwq, bwo, o_hbm,
               kv, xbuf, wqbuf, wobuf, acc, obuf, kvsem, xsem, wsem, osem):
        xs, ks, vs, wqs, wos = (ax, bx), (ak, bk), (av, bv), (awq, bwq), (awo, bwo)

        def kv_start(s, br, jb, n, sem):
            g, half = s // NH, s % NH
            bs = pl.ds(half * NB + jb, n)
            hs = pl.ds(g * C, C)
            pltpu.make_async_copy(ks[br].at[bs, hs], kv.at[s % 2, br, 0, pl.ds(jb, n)], sem).start()
            pltpu.make_async_copy(vs[br].at[bs, hs], kv.at[s % 2, br, 1, pl.ds(jb, n)], sem).start()

        def wq_copy(g, br):
            cs = pl.ds(pl.multiple_of(g * CW, CW), CW)
            return pltpu.make_async_copy(wqs[br].at[:, cs], wqbuf.at[g % 2, br], wsem.at[g % 2, br, 0])

        def wo_copy(g, br):
            cs = pl.ds(pl.multiple_of(g * CW, CW), CW)
            return pltpu.make_async_copy(wos[br].at[cs, :], wobuf.at[g % 2, br], wsem.at[g % 2, br, 1])

        def o_copy(br, b):
            return pltpu.make_async_copy(obuf.at[br, b], o_hbm.at[b, :, pl.ds(br * D, D)], osem.at[br, b])

        def small_coords(i):
            s = i // SPB
            r = i % SPB
            return s, r // HB, (r % HB) * SM

        def pro(i, carry):
            s, br, jb = small_coords(i)
            b0 = s * NB + jb
            for brs in range(2):
                @pl.when(br == brs)
                def _():
                    pltpu.make_async_copy(xs[brs].at[pl.ds(b0, SM)], xbuf.at[brs, pl.ds(b0, SM)], xsem.at[i]).start()
                @pl.when(i == brs * HB)
                def _():
                    wq_copy(0, brs).start()
                @pl.when(br == brs)
                def _():
                    kv_start(s, brs, jb, SM, kvsem.at[2 + i])
                @pl.when(i == brs * HB)
                def _():
                    wo_copy(0, brs).start()
            return carry
        lax.fori_loop(0, 2 * SPB, pro, 0)

        def run_chunks(chunks, g, top):
            wp = g % 2

            def qproj(k):
                p, br, jb, b = chunks[k]
                q = jnp.dot(xbuf[br, b], wqbuf[wp, br], preferred_element_type=f32)
                return (q * c).astype(bf16)

            def qk(q, k, hl):
                p, br, jb, b = chunks[k]
                qh = q[:, hl * DH:(hl + 1) * DH]
                return lax.dot_general(qh, kv[p, br, 0, jb, hl], (((1,), (1,)), ((), ())), preferred_element_type=f32)

            def recip(l):
                return 1.0 / l if rcp == "div" else pl.reciprocal(l, approx=True)

            def softmax(s):
                m = jnp.max(s, axis=-1, keepdims=True)
                p = jnp.exp2(s - m)
                l = jnp.sum(p, axis=-1, keepdims=True)
                if prenorm:
                    return (p * recip(l)).astype(bf16), None
                return p.astype(bf16), l

            def pv(pp, l, k, hl):
                p, br, jb, b = chunks[k]
                o = jnp.dot(pp, kv[p, br, 1, jb, hl], preferred_element_type=f32)
                if prenorm:
                    return o.astype(bf16)
                return (o * recip(l)).astype(bf16)

            def oproj(os_, k):
                p, br, jb, b = chunks[k]
                og = jnp.concatenate(os_, axis=-1)
                r = jnp.dot(og, wobuf[wp, br], preferred_element_type=f32)
                new = jnp.where(g > 0, acc[br, b], 0.0) + r
                acc[br, b] = new
                obuf[br, b] = new.astype(bf16)
                @pl.when(g == NG - 1)
                def _():
                    o_copy(br, b).start()

            top()
            n = len(chunks) * C
            Q = {}; S = {}; P = {}; O = {k: [] for k in range(len(chunks))}
            for t in range(-1 - qlead, n + 1):
                tq = t + 1 + qlead
                if 0 <= tq < n and tq % C == 0:
                    Q[tq // C] = qproj(tq // C)
                if 0 <= t + 1 < n:
                    k, hl = divmod(t + 1, C)
                    S[t + 1] = qk(Q[k], k, hl)
                if 0 <= t < n:
                    P[t] = softmax(S.pop(t))
                if 0 <= t - 1 < n:
                    k, hl = divmod(t - 1, C)
                    pp, l = P.pop(t - 1)
                    O[k].append(pv(pp, l, k, hl))
                    if len(O[k]) == C:
                        oproj(O[k], k)

        def small_body(i, carry):
            s, br, jb = small_coords(i)
            g, half = s // NH, s % NH
            b0 = half * NB + jb
            p = s % 2

            def top():
                ip = jnp.maximum(i - 1, 0)
                sp, brp, jp = small_coords(ip)
                sn = sp + 2
                sem = kvsem.at[jnp.where(sn < SP, 2 + ip + 2 * SPB, sn % 2)]
                for brs in range(2):
                    @pl.when(jnp.logical_and(jnp.logical_and(i >= 1, sn <= SP), brp == brs))
                    def _():
                        kv_start(sn, brs, jp, SM, sem)
                for brs in range(2):
                    @pl.when(i == 1 + brs)
                    def _():
                        wq_copy(1, brs).start()
                        wo_copy(1, brs).start()
                for kvi in range(2):
                    sl = kv.at[p, br, kvi, pl.ds(jb, SM)]
                    pltpu.make_async_copy(sl, sl, kvsem.at[2 + i]).wait()
                @pl.when(s < 2)
                def _():
                    xl = xbuf.at[br, pl.ds(b0, SM)]
                    pltpu.make_async_copy(xl, xl, xsem.at[jnp.minimum(i, 2 * SPB - 1)]).wait()
                @pl.when(jnp.logical_and(half == 0, jb == 0))
                def _():
                    wl = wqbuf.at[g % 2, br]
                    pltpu.make_async_copy(wl, wl, wsem.at[g % 2, br, 0]).wait()
                    pltpu.make_async_copy(wl, wl, wsem.at[g % 2, br, 1]).wait()

            run_chunks([(p, br, jb + jj, b0 + jj) for jj in range(SM)], g, top)
            return carry

        lax.fori_loop(0, NSM, small_body, 0)

        def big_body(s, carry):
            g, half = s // NH, s % NH
            p = s % 2

            def top():
                @pl.when(s + 1 < NS)
                def _():
                    for br in range(2):
                        kv_start(s + 1, br, 0, NB, kvsem.at[1 - p])
                for br in range(2):
                    @pl.when(jnp.logical_and(half == NH - 1, g + 1 < NG))
                    def _():
                        wq_copy(g + 1, br).start()
                        wo_copy(g + 1, br).start()
                sl = kv.at[p]
                pltpu.make_async_copy(sl, sl, kvsem.at[p]).wait()
                @pl.when(half == 0)
                def _():
                    for br in range(2):
                        wq_copy(g, br).wait()
                        wo_copy(g, br).wait()

            run_chunks([(p, br, jb, half * NB + jb) for br in range(2) for jb in range(NB)], g, top)
            return carry

        lax.fori_loop(SP, NS, big_body, 0)

        for br in range(2):
            for b in range(B):
                o_copy(br, b).wait()

    any_spec = pl.BlockSpec(memory_space=pl.ANY)
    scratch = [
        pltpu.VMEM((2, 2, 2, NB, C, SK, DH), bf16),
        pltpu.VMEM((2, B, SQ, D), bf16),
        pltpu.VMEM((2, 2, D, CW), bf16),
        pltpu.VMEM((2, 2, CW, D), bf16),
        pltpu.VMEM((2, B, SQ, D), f32),
        pltpu.VMEM((2, B, SQ, D), bf16),
        pltpu.SemaphoreType.DMA((2 + NSM,)),
        pltpu.SemaphoreType.DMA((2 * SPB,)),
        pltpu.SemaphoreType.DMA((2, 2, 2)),
        pltpu.SemaphoreType.DMA((2, B)),
    ]

    def fn(A_x, A_k_cache, A_v_cache, A_wq, A_wo, B_x, B_k_cache, B_v_cache, B_wq, B_wo):
        return pl.pallas_call(
            kernel,
            in_specs=[any_spec] * 10,
            out_specs=any_spec,
            out_shape=jax.ShapeDtypeStruct((B, SQ, 2 * D), jnp.bfloat16),
            scratch_shapes=scratch,
            interpret=interpret,
            compiler_params=pltpu.CompilerParams(
                vmem_limit_bytes=110 * 1024 * 1024, disable_bounds_checks=nobounds),
        )(A_x, A_k_cache, A_v_cache, A_wq, A_wo, B_x, B_k_cache, B_v_cache, B_wq, B_wo)
    return fn


_impl = make(SP=3)


@jax.jit
def pallas_concat_heads__mha_block_cached__mha_block_cached__near_ridge_kernel(
    A_x: jax.Array,
    A_k_cache: jax.Array,
    A_v_cache: jax.Array,
    A_wq: jax.Array,
    A_wo: jax.Array,
    B_x: jax.Array,
    B_k_cache: jax.Array,
    B_v_cache: jax.Array,
    B_wq: jax.Array,
    B_wo: jax.Array,
):
    return _impl(A_x, A_k_cache, A_v_cache, A_wq, A_wo, B_x, B_k_cache, B_v_cache, B_wq, B_wo)
```

```python
import jax
import jax.numpy as jnp
from jax import lax
import jax.experimental.pallas as pl
import jax.experimental.pallas.tpu as pltpu

LOG2E = 1.4426950408889634
BF16 = jnp.bfloat16
F32 = jnp.float32

C = 4
NB = 8
QS = 4
SLAG = 1
PLAG = 1
OLAG = 2


def _build(B, SQ, D, H, SK, DH):
    NG = H // C
    NH = B // NB
    assert NH == 2 and NG >= 2 and B % QS == 0 and QS >= 2
    NS = NG * NH
    CW = C * DH
    QPB = B // QS
    NQS = 2 * QPB
    c = (DH ** -0.5) * LOG2E

    def kernel(ax, ak, av, awq, awo, bx, bk, bv, bwq, bwo, o_hbm,
               kv, xbuf, qbuf, wqbuf, wobuf, acc, obuf, kvsem, xsem, wqsem, wosem, osem):
        xs, ks, vs, wqs, wos = (ax, bx), (ak, bk), (av, bv), (awq, bwq), (awo, bwo)

        def kv_start(s, br):
            g, half = lax.shift_right_logical(s, 1), s & 1
            bs = pl.ds(half * NB, NB)
            hs = pl.ds(g * C, C)
            pltpu.make_async_copy(ks[br].at[bs, hs], kv.at[half, br, 0], kvsem.at[br, half]).start()
            pltpu.make_async_copy(vs[br].at[bs, hs], kv.at[half, br, 1], kvsem.at[br, half]).start()

        def kv_wait(half, br):
            both = kv.at[half, br]
            pltpu.make_async_copy(both, both, kvsem.at[br, half]).wait()

        def x_copy(br, b0, nb, sem):
            return pltpu.make_async_copy(xs[br].at[pl.ds(b0, nb)], xbuf.at[br, pl.ds(b0, nb)], sem)

        def wq_copy(g, br):
            cs = pl.ds(pl.multiple_of(g * CW, CW), CW)
            return pltpu.make_async_copy(wqs[br].at[:, cs], wqbuf.at[g & 1, br], wqsem.at[g & 1, br])

        def wo_copy(g, br):
            cs = pl.ds(pl.multiple_of(g * CW, CW), CW)
            return pltpu.make_async_copy(wos[br].at[cs, :], wobuf.at[g & 1, br], wosem.at[g & 1, br])

        def o_copy(br, b):
            return pltpu.make_async_copy(obuf.at[br, b], o_hbm.at[b, :, pl.ds(br * D, D)], osem.at[br, b])

        def issue_x(i, carry):
            ii = jnp.maximum(i - 1, 0)
            br = lax.div(ii, QPB)
            b0 = lax.rem(ii, QPB) * QS

            @pl.when(i == 0)
            def _():
                wq_copy(0, 0).start()
                x_copy(0, 0, 1, xsem.at[NQS]).start()

            @pl.when(i == 1)
            def _():
                x_copy(0, 1, QS - 1, xsem.at[0]).start()

            for brs in range(2):
                @pl.when(jnp.logical_and(i >= 2, br == brs))
                def _():
                    x_copy(brs, b0, QS, xsem.at[ii]).start()

            @pl.when(i == 1 + QPB)
            def _():
                wq_copy(0, 1).start()
            return carry

        lax.fori_loop(0, NQS + 1, issue_x, 0)

        def issue_rest(i, carry):
            @pl.when(i == 0)
            def _():
                for br in range(2):
                    wq_copy(1, br).start()

            @pl.when(i == 1)
            def _():
                for br in range(2):
                    wo_copy(0, br).start()

            for br in range(2):
                @pl.when(i >= 2)
                def _():
                    kv_start(i - 2, br)
            return carry

        lax.fori_loop(0, 4, issue_rest, 0)

        def qproj(slot, br, b):
            q = jnp.dot(xbuf[br, b], wqbuf[slot, br], preferred_element_type=F32)
            qbuf[slot, br, b] = (q * c).astype(BF16)

        x_copy(0, 0, 1, xsem.at[NQS]).wait()
        wq_copy(0, 0).wait()
        qproj(0, 0, 0)
        x_copy(0, 1, QS - 1, xsem.at[0]).wait()
        for j in range(1, QS):
            qproj(0, 0, j)

        def q_small(i, carry):
            br = lax.div(i, QPB)
            b0 = lax.rem(i, QPB) * QS
            xl = xbuf.at[br, pl.ds(b0, QS)]
            pltpu.make_async_copy(xl, xl, xsem.at[i]).wait()

            @pl.when(i == QPB)
            def _():
                wq_copy(0, 1).wait()

            for j in range(QS):
                qproj(0, br, b0 + j)
            return carry

        lax.fori_loop(1, NQS, q_small, 0)

        def q_body(g):
            for br in range(2):
                wq_copy(g, br).wait()
            for br in range(2):
                for b in range(B):
                    qproj(g & 1, br, b)

        def attn_body(s, carry):
            g, half = lax.shift_right_logical(s, 1), s & 1
            gp = g & 1
            chunks = [(br, jb, half * NB + jb) for br in range(2) for jb in range(NB)]

            for br in range(2):
                kv_wait(half, br)

            @pl.when(half == 0)
            def _():
                for br in range(2):
                    wo_copy(g, br).wait()

            def qk(k, hl):
                br, jb, b = chunks[k]
                qh = qbuf[gp, br, b, :, hl * DH:(hl + 1) * DH]
                return lax.dot_general(qh, kv[half, br, 0, jb, hl], (((1,), (1,)), ((), ())),
                                       preferred_element_type=F32)

            def softmax(sc):
                m = jnp.max(sc, axis=-1, keepdims=True)
                p = jnp.exp2(sc - m)
                return p.astype(BF16), jnp.sum(p, axis=-1, keepdims=True)

            def pv(p, l, k, hl):
                br, jb, b = chunks[k]
                o = jnp.dot(p, kv[half, br, 1, jb, hl], preferred_element_type=F32)
                r = pl.reciprocal(l, approx=True)
                r = r * (2.0 - l * r)
                return (o * r).astype(BF16)

            def oproj(heads, k):
                br, jb, b = chunks[k]
                r = jnp.dot(jnp.concatenate(heads, axis=-1), wobuf[gp, br], preferred_element_type=F32)
                new = jnp.where(g > 0, acc[br, b], 0.0) + r
                acc[br, b] = new
                obuf[br, b] = new.astype(BF16)

                @pl.when(g == NG - 1)
                def _():
                    o_copy(br, b).start()

            def refill(br):
                @pl.when(s + 2 < NS)
                def _():
                    kv_start(s + 2, br)

            n = len(chunks) * C
            scores, probs = {}, {}
            heads = {k: [] for k in range(len(chunks))}
            pending = []
            for t in range(-SLAG, n + PLAG + OLAG + 1):
                if 0 <= t + SLAG < n:
                    scores[t + SLAG] = qk(*divmod(t + SLAG, C))
                if 0 <= t < n:
                    probs[t] = softmax(scores.pop(t))
                if 0 <= t - PLAG < n:
                    k, hl = divmod(t - PLAG, C)
                    heads[k].append(pv(*probs.pop(t - PLAG), k, hl))
                    if hl == C - 1:
                        pending.append((t + OLAG, k))
                    if t - PLAG == n // 2 - 1:
                        refill(0)
                while pending and pending[0][0] <= t:
                    k = pending.pop(0)[1]
                    oproj(heads[k], k)
            refill(1)

            for br in range(2):
                @pl.when(jnp.logical_and(half == 0, g + 2 < NG))
                def _():
                    wq_copy(g + 2, br).start()

                @pl.when(jnp.logical_and(half == 0, g + 1 < NG))
                def _():
                    wo_copy(g + 1, br).start()
            return carry

        def group(gm, carry):
            g = gm - 1
            lax.fori_loop(jnp.where(g >= 0, 2 * g, 0), jnp.where(g >= 0, 2 * g + 2, 0), attn_body, 0)

            @pl.when(g + 2 < NG)
            def _():
                q_body(g + 2)
            return carry

        lax.fori_loop(0, NG + 1, group, 0)

        for br in range(2):
            for b in range(B):
                o_copy(br, b).wait()

    scratch = [
        pltpu.VMEM((2, 2, 2, NB, C, SK, DH), BF16),
        pltpu.VMEM((2, B, SQ, D), BF16),
        pltpu.VMEM((2, 2, B, SQ, CW), BF16),
        pltpu.VMEM((2, 2, D, CW), BF16),
        pltpu.VMEM((2, 2, CW, D), BF16),
        pltpu.VMEM((2, B, SQ, D), F32),
        pltpu.VMEM((2, B, SQ, D), BF16),
        pltpu.SemaphoreType.DMA((2, 2)),
        pltpu.SemaphoreType.DMA((NQS + 1,)),
        pltpu.SemaphoreType.DMA((2, 2)),
        pltpu.SemaphoreType.DMA((2, 2)),
        pltpu.SemaphoreType.DMA((2, B)),
    ]
    return kernel, scratch


@jax.jit
def pallas_concat_heads__mha_block_cached__mha_block_cached__near_ridge_kernel(
    A_x: jax.Array,
    A_k_cache: jax.Array,
    A_v_cache: jax.Array,
    A_wq: jax.Array,
    A_wo: jax.Array,
    B_x: jax.Array,
    B_k_cache: jax.Array,
    B_v_cache: jax.Array,
    B_wq: jax.Array,
    B_wo: jax.Array,
):
    B, SQ, D = A_x.shape
    _, H, SK, DH = A_k_cache.shape
    kernel, scratch = _build(B, SQ, D, H, SK, DH)
    hbm = pl.BlockSpec(memory_space=pl.ANY)
    return pl.pallas_call(
        kernel,
        in_specs=[hbm] * 10,
        out_specs=hbm,
        out_shape=jax.ShapeDtypeStruct((B, SQ, 2 * D), BF16),
        scratch_shapes=scratch,
        compiler_params=pltpu.CompilerParams(
            vmem_limit_bytes=110 * 1024 * 1024,
            disable_bounds_checks=True,
        ),
    )(A_x, A_k_cache, A_v_cache, A_wq, A_wo, B_x, B_k_cache, B_v_cache, B_wq, B_wo)
```

```python
import jax
import jax.numpy as jnp
from jax import lax
import jax.experimental.pallas as pl
import jax.experimental.pallas.tpu as pltpu

LOG2E = 1.4426950408889634
BF16 = jnp.bfloat16
F32 = jnp.float32

C = 4
NB = 8
QS = 4
QM = 4
SLAG = 1
PLAG = 1
OLAG = 2


def _build(B, SQ, D, H, SK, DH):
    NG = H // C
    NH = B // NB
    assert NH == 2 and NG >= 2 and B % QS == 0 and QS >= 2 and B % QM == 0
    NS = NG * NH
    CW = C * DH
    QPB = B // QS
    NQS = 2 * QPB
    c = (DH ** -0.5) * LOG2E

    def kernel(ax, ak, av, awq, awo, bx, bk, bv, bwq, bwo, o_hbm,
               kv, xbuf, qbuf, wqbuf, wobuf, acc, obuf, kvsem, xsem, wqsem, wosem, osem):
        xs, ks, vs, wqs, wos = (ax, bx), (ak, bk), (av, bv), (awq, bwq), (awo, bwo)

        def kv_start(s, br):
            g, half = lax.shift_right_logical(s, 1), s & 1
            bs = pl.ds(half * NB, NB)
            hs = pl.ds(g * C, C)
            pltpu.make_async_copy(ks[br].at[bs, hs], kv.at[half, br, 0], kvsem.at[br, half]).start()
            pltpu.make_async_copy(vs[br].at[bs, hs], kv.at[half, br, 1], kvsem.at[br, half]).start()

        def kv_wait(half, br):
            both = kv.at[half, br]
            pltpu.make_async_copy(both, both, kvsem.at[br, half]).wait()

        def x_copy(br, b0, nb, sem):
            return pltpu.make_async_copy(xs[br].at[pl.ds(b0, nb)], xbuf.at[br, pl.ds(b0, nb)], sem)

        def wq_copy(g, br):
            cs = pl.ds(pl.multiple_of(g * CW, CW), CW)
            return pltpu.make_async_copy(wqs[br].at[:, cs], wqbuf.at[g & 1, br], wqsem.at[g & 1, br])

        def wo_copy(g, br):
            cs = pl.ds(pl.multiple_of(g * CW, CW), CW)
            return pltpu.make_async_copy(wos[br].at[cs, :], wobuf.at[g & 1, br], wosem.at[g & 1, br])

        def o_copy(br, b):
            return pltpu.make_async_copy(obuf.at[br, b], o_hbm.at[b, :, pl.ds(br * D, D)], osem.at[br, b])

        def issue_x(i, carry):
            ii = jnp.maximum(i - 1, 0)
            br = lax.div(ii, QPB)
            b0 = lax.rem(ii, QPB) * QS

            @pl.when(i == 0)
            def _():
                wq_copy(0, 0).start()
                x_copy(0, 0, 1, xsem.at[NQS]).start()

            @pl.when(i == 1)
            def _():
                x_copy(0, 1, QS - 1, xsem.at[0]).start()

            for brs in range(2):
                @pl.when(jnp.logical_and(i >= 2, br == brs))
                def _():
                    x_copy(brs, b0, QS, xsem.at[ii]).start()

            @pl.when(i == 1 + QPB)
            def _():
                wq_copy(0, 1).start()
            return carry

        lax.fori_loop(0, NQS + 1, issue_x, 0)

        def issue_rest(i, carry):
            @pl.when(i == 0)
            def _():
                for br in range(2):
                    wq_copy(1, br).start()

            @pl.when(i == 1)
            def _():
                for br in range(2):
                    wo_copy(0, br).start()

            for br in range(2):
                @pl.when(i >= 2)
                def _():
                    kv_start(i - 2, br)
            return carry

        lax.fori_loop(0, 4, issue_rest, 0)

        def qproj(slot, br, b0, nb=1):
            x = xbuf[br, pl.ds(b0, nb)].reshape(nb * SQ, D)
            q = jnp.dot(x, wqbuf[slot, br], preferred_element_type=F32)
            qbuf[slot, br, pl.ds(b0, nb)] = (q * c).astype(BF16).reshape(nb, SQ, CW)

        x_copy(0, 0, 1, xsem.at[NQS]).wait()
        wq_copy(0, 0).wait()
        qproj(0, 0, 0)
        x_copy(0, 1, QS - 1, xsem.at[0]).wait()
        for j in range(1, QS):
            qproj(0, 0, j)

        def q_small(i, carry):
            br = lax.div(i, QPB)
            b0 = lax.rem(i, QPB) * QS
            xl = xbuf.at[br, pl.ds(b0, QS)]
            pltpu.make_async_copy(xl, xl, xsem.at[i]).wait()

            @pl.when(i == QPB)
            def _():
                wq_copy(0, 1).wait()

            for j in range(QS):
                qproj(0, br, b0 + j)
            return carry

        lax.fori_loop(1, NQS, q_small, 0)

        def q_body(g):
            for br in range(2):
                wq_copy(g, br).wait()
            for br in range(2):
                for b in range(0, B, QM):
                    qproj(g & 1, br, b, QM)

        def attn_body(s, carry):
            g, half = lax.shift_right_logical(s, 1), s & 1
            gp = g & 1
            chunks = [(br, jb, half * NB + jb) for br in range(2) for jb in range(NB)]

            for br in range(2):
                kv_wait(half, br)

            @pl.when(half == 0)
            def _():
                for br in range(2):
                    wo_copy(g, br).wait()

            def qk(k, hl):
                br, jb, b = chunks[k]
                qh = qbuf[gp, br, b, :, hl * DH:(hl + 1) * DH]
                return lax.dot_general(qh, kv[half, br, 0, jb, hl], (((1,), (1,)), ((), ())),
                                       preferred_element_type=F32)

            def softmax(sc):
                m = jnp.max(sc, axis=-1, keepdims=True)
                p = jnp.exp2(sc - m)
                return p.astype(BF16), jnp.sum(p, axis=-1, keepdims=True)

            def pv(p, l, k, hl):
                br, jb, b = chunks[k]
                o = jnp.dot(p, kv[half, br, 1, jb, hl], preferred_element_type=F32)
                r = pl.reciprocal(l, approx=True)
                r = r * (2.0 - l * r)
                return (o * r).astype(BF16)

            def oproj(heads, k):
                br, jb, b = chunks[k]
                r = jnp.dot(jnp.concatenate(heads, axis=-1), wobuf[gp, br], preferred_element_type=F32)
                new = jnp.where(g > 0, acc[br, b], 0.0) + r
                acc[br, b] = new
                obuf[br, b] = new.astype(BF16)

                @pl.when(g == NG - 1)
                def _():
                    o_copy(br, b).start()

            def refill(br):
                @pl.when(s + 2 < NS)
                def _():
                    kv_start(s + 2, br)

            n = len(chunks) * C
            scores, probs = {}, {}
            heads = {k: [] for k in range(len(chunks))}
            pending = []
            for t in range(-SLAG, n + PLAG + OLAG + 1):
                if 0 <= t + SLAG < n:
                    scores[t + SLAG] = qk(*divmod(t + SLAG, C))
                if 0 <= t < n:
                    probs[t] = softmax(scores.pop(t))
                if 0 <= t - PLAG < n:
                    k, hl = divmod(t - PLAG, C)
                    heads[k].append(pv(*probs.pop(t - PLAG), k, hl))
                    if hl == C - 1:
                        pending.append((t + OLAG, k))
                    if t - PLAG == n // 2 - 1:
                        refill(0)
                while pending and pending[0][0] <= t:
                    k = pending.pop(0)[1]
                    oproj(heads[k], k)
            refill(1)

            for br in range(2):
                @pl.when(jnp.logical_and(half == 0, g + 2 < NG))
                def _():
                    wq_copy(g + 2, br).start()

                @pl.when(jnp.logical_and(half == 0, g + 1 < NG))
                def _():
                    wo_copy(g + 1, br).start()
            return carry

        def group(gm, carry):
            g = gm - 1
            lax.fori_loop(jnp.where(g >= 0, 2 * g, 0), jnp.where(g >= 0, 2 * g + 2, 0), attn_body, 0)

            @pl.when(g + 2 < NG)
            def _():
                q_body(g + 2)
            return carry

        lax.fori_loop(0, NG + 1, group, 0)

        for br in range(2):
            for b in range(B):
                o_copy(br, b).wait()

    scratch = [
        pltpu.VMEM((2, 2, 2, NB, C, SK, DH), BF16),
        pltpu.VMEM((2, B, SQ, D), BF16),
        pltpu.VMEM((2, 2, B, SQ, CW), BF16),
        pltpu.VMEM((2, 2, D, CW), BF16),
        pltpu.VMEM((2, 2, CW, D), BF16),
        pltpu.VMEM((2, B, SQ, D), F32),
        pltpu.VMEM((2, B, SQ, D), BF16),
        pltpu.SemaphoreType.DMA((2, 2)),
        pltpu.SemaphoreType.DMA((NQS + 1,)),
        pltpu.SemaphoreType.DMA((2, 2)),
        pltpu.SemaphoreType.DMA((2, 2)),
        pltpu.SemaphoreType.DMA((2, B)),
    ]
    return kernel, scratch


@jax.jit
def pallas_concat_heads__mha_block_cached__mha_block_cached__near_ridge_kernel(
    A_x: jax.Array,
    A_k_cache: jax.Array,
    A_v_cache: jax.Array,
    A_wq: jax.Array,
    A_wo: jax.Array,
    B_x: jax.Array,
    B_k_cache: jax.Array,
    B_v_cache: jax.Array,
    B_wq: jax.Array,
    B_wo: jax.Array,
):
    B, SQ, D = A_x.shape
    _, H, SK, DH = A_k_cache.shape
    kernel, scratch = _build(B, SQ, D, H, SK, DH)
    hbm = pl.BlockSpec(memory_space=pl.ANY)
    return pl.pallas_call(
        kernel,
        in_specs=[hbm] * 10,
        out_specs=hbm,
        out_shape=jax.ShapeDtypeStruct((B, SQ, 2 * D), BF16),
        scratch_shapes=scratch,
        compiler_params=pltpu.CompilerParams(
            vmem_limit_bytes=110 * 1024 * 1024,
            disable_bounds_checks=True,
        ),
    )(A_x, A_k_cache, A_v_cache, A_wq, A_wo, B_x, B_k_cache, B_v_cache, B_wq, B_wo)
```
